```python
import jax
import jax.numpy as jnp

def _softmax(x, axis=-1):
    return jax.nn.softmax(x, axis=axis)

def _gelu(x):
    return jax.nn.gelu(x, approximate=True)

def _silu(x):
    return jax.nn.silu(x)

def _sigmoid(x):
    return jax.nn.sigmoid(x)

def _layernorm(x, axis=-1, eps=1e-05):
    m = jnp.mean(x, axis=axis, keepdims=True)
    v = jnp.var(x, axis=axis, keepdims=True)
    return (x - m) / jnp.sqrt(v + eps)

def _scatter_add(tgt, idx, src, axis=0):
    return tgt.at[idx].add(src)

def _segment_sum(src, seg, n):
    return jax.ops.segment_sum(src, seg, n)

class _Rng:

    def __init__(self, key):
        self._k = key

    def _next(self):
        self._k, sub = jax.random.split(self._k)
        return sub

    def normal(self, shape):
        return jax.random.normal(self._next(), shape, dtype=jnp.bfloat16)

    def randint(self, lo, hi, shape):
        return jax.random.randint(self._next(), shape, lo, hi, dtype=jnp.int32)

    def uniform(self, shape, lo=0.0, hi=1.0):
        return jax.random.uniform(self._next(), shape, jnp.bfloat16, lo, hi)

    def permutation(self, n):
        return jax.random.permutation(self._next(), n)
kernel_name = 'concat_heads__compressed_kv_cla__memory_aug_recurrent_mem_tr__prompt'

def setup_inputs():
    _rng = _Rng(jax.random.key(int.from_bytes(__import__("os").urandom(4), "little")))
    _w = lambda a: (lambda t: t.astype(jnp.bfloat16) if jnp.issubdtype(t.dtype, jnp.floating) else t)(jnp.asarray(a))

    def _A_setup():
        B, H, Sq, Sk, D, M = (1, 32, 2048, 2048, 128, 576)
        Dc = 4 * D
        return {'x': _w((lambda *s: _rng.normal(s) * 0.05)(B, Sq, M)), 'c_kv': _w((lambda *s: _rng.normal(s) * 0.05)(B, Sk, Dc)), 'w_q': _w((lambda *s: _rng.normal(s) * 0.05)(M, H, D) * M ** (-0.5)), 'w_uk': _w((lambda *s: _rng.normal(s) * 0.05)(Dc, H, D) * Dc ** (-0.5)), 'w_uv': _w((lambda *s: _rng.normal(s) * 0.05)(Dc, H, D) * Dc ** (-0.5)), 'w_o': _w((lambda *s: _rng.normal(s) * 0.05)(H, D, M) * (H * D) ** (-0.5))}
    _A_in = _A_setup()

    def _B_setup():
        B, S, Dm = (1, 2048, 576)
        H, Dh = (32, 128)
        M, seg = (8, 32)
        seg = min(seg, S)
        S = S // seg * seg
        return {'x': _w((lambda *s: _rng.normal(s) * 0.05)(B, S, Dm)), 'mem0': _w((lambda *s: _rng.normal(s) * 0.05)(B, M, Dm)), 'Wq': _w((lambda *s: _rng.normal(s) * 0.05)(Dm, H, Dh) * Dm ** (-0.5)), 'Wk': _w((lambda *s: _rng.normal(s) * 0.05)(Dm, H, Dh) * Dm ** (-0.5)), 'Wv': _w((lambda *s: _rng.normal(s) * 0.05)(Dm, H, Dh) * Dm ** (-0.5)), 'Wo': _w((lambda *s: _rng.normal(s) * 0.05)(H, Dh, Dm) * (H * Dh) ** (-0.5)), 'seg_len': seg}
    _B_in = _B_setup()
    return {'A_x': _A_in['x'], 'A_c_kv': _A_in['c_kv'], 'A_w_q': _A_in['w_q'], 'A_w_uk': _A_in['w_uk'], 'A_w_uv': _A_in['w_uv'], 'A_w_o': _A_in['w_o'], 'B_x': _B_in['x'], 'B_mem0': _B_in['mem0'], 'B_Wq': _B_in['Wq'], 'B_Wk': _B_in['Wk'], 'B_Wv': _B_in['Wv'], 'B_Wo': _B_in['Wo'], 'B_seg_len': _B_in['seg_len']}

def reference(A_x, A_c_kv, A_w_q, A_w_uk, A_w_uv, A_w_o, B_x, B_mem0, B_Wq, B_Wk, B_Wv, B_Wo, B_seg_len):

    def _A_ref(x, c_kv, w_q, w_uk, w_uv, w_o):
        B, Sq, M = (x.shape[0], x.shape[1], x.shape[2])
        Sk = c_kv.shape[1]
        H, D = (w_q.shape[1], w_q.shape[2])
        q = jnp.einsum('bqm,mhd->bhqd', x, w_q)
        k = jnp.einsum('bkc,chd->bhkd', c_kv, w_uk)
        v = jnp.einsum('bkc,chd->bhkd', c_kv, w_uv)
        scores = jnp.einsum('bhqd,bhkd->bhqk', q, k) * D ** (-0.5)
        off = Sk - Sq
        qi = jnp.arange(Sq)[:, None]
        kj = jnp.arange(Sk)[None, :]
        cmask = kj <= qi + off
        scores = jnp.where(cmask[None, None], scores, -1000000000.0)
        p = _softmax(scores, axis=-1)
        ctx = jnp.einsum('bhqk,bhkd->bhqd', p, v)
        return jnp.einsum('bhqd,hdm->bqm', ctx, w_o)

    def _B_ref(x, mem0, Wq, Wk, Wv, Wo, seg_len):
        B, S, Dm = x.shape
        H, Dh = (Wq.shape[1], Wq.shape[2])
        M = mem0.shape[1]
        scale = Dh ** (-0.5)
        n_seg = S // seg_len
        L = M + seg_len
        idx = jnp.arange(L)
        mask = (idx[:, None] < M) | (idx[:, None] >= idx[None, :])
        mem = mem0
        outs = []
        for s in range(n_seg):
            xs = x[:, s * seg_len:(s + 1) * seg_len, :].copy()
            h = jnp.concatenate([mem, xs], axis=1)
            q = jnp.einsum('btd,dhe->bhte', h, Wq)
            k = jnp.einsum('btd,dhe->bhte', h, Wk)
            v = jnp.einsum('btd,dhe->bhte', h, Wv)
            scores = jnp.einsum('bhqe,bhke->bhqk', q, k) * scale
            scores = jnp.where(mask[None, None], scores, -1000000000.0)
            p = _softmax(scores, axis=-1)
            o = jnp.einsum('bhqk,bhke->bhqe', p, v)
            o = jnp.einsum('bhte,hed->btd', o, Wo)
            mem = o[:, :M, :].copy()
            outs.append(o[:, M:, :])
        return jnp.concatenate(outs, axis=1)
    a = _A_ref(A_x, A_c_kv, A_w_q, A_w_uk, A_w_uv, A_w_o)
    b = _B_ref(B_x, B_mem0, B_Wq, B_Wk, B_Wv, B_Wo, B_seg_len)
    return jnp.concatenate([a, b], axis=-1)
```

```python
import functools

import jax
import jax.numpy as jnp
import numpy as np
import jax.experimental.pallas as pl
import jax.experimental.pallas.tpu as pltpu

_H = 32
_D = 128
_S = 2048
_DM = 576
_DC = 512
_MEM = 8
_SEG = 32
_NSEG = _S // _SEG
_L = _SEG + _MEM
_LP = 48
_BQ = 512
_LOG2E = 1.4426950408889634
_QSCALE = float(_D ** -0.5) * _LOG2E
_NEG_REF = -1000000000.0 * _LOG2E
_NEG_OUT = -1e30

_NT = (((1,), (1,)), ((), ()))
_F32 = jnp.float32
_BF16 = jnp.bfloat16


def _dot(a, b):
    return jnp.dot(a, b, preferred_element_type=_F32)


def _dot_nt(a, b):
    return jax.lax.dot_general(a, b, _NT, preferred_element_type=_F32)


def _relayout(src_ref, dst_ref, k):
    def body(c, _):
        r = pl.multiple_of(c * 64, 64)
        for u in range(4):
            blk = src_ref[pl.ds(r + u * 16, 16)]
            dst_ref[:, pl.ds(r + u * 16, 16), :] = jnp.swapaxes(blk, 0, 1)
    jax.lax.fori_loop(0, k // 64, body, None)


def _b_bias(nheads):
    r = jax.lax.broadcasted_iota(jnp.int32, (128, 128), 0)
    c = jax.lax.broadcasted_iota(jnp.int32, (128, 128), 1)
    rh = (r >= _L).astype(jnp.int32) + (r >= 2 * _L).astype(jnp.int32) + (r >= 3 * _L).astype(jnp.int32)
    ch = (c >= _L).astype(jnp.int32) + (c >= 2 * _L).astype(jnp.int32) + (c >= 3 * _L).astype(jnp.int32)
    ri = r - rh * _L
    ci = c - ch * _L
    same = rh == ch
    ok = jnp.logical_or(jnp.logical_or(ri >= _SEG, ci >= _SEG), ci <= ri)
    valid = jnp.logical_and(same, ok)
    fill = jnp.where(same, _NEG_REF, _NEG_OUT).astype(_F32)
    return valid, fill


def _b_step(s, mem, xb_ref, wq_ref, wk_ref, wv_ref, wo_ref, out_ref, valid, fill):
    r0 = pl.multiple_of(s * _SEG, _SEG)
    xs = xb_ref[pl.ds(r0, _SEG), :]
    memb = jnp.concatenate([mem, jnp.zeros_like(mem)], axis=0).astype(_BF16)
    h = jnp.concatenate([xs, memb], axis=0)
    acc = None
    zpad = jnp.zeros((8, _D), _F32)
    for g0 in range(0, _H, 3):
        heads = list(range(g0, min(g0 + 3, _H)))

        def stack(w_ref, scale=None):
            parts = [_dot(h, w_ref[hh])[0:_L] for hh in heads]
            parts += [jnp.zeros((_L, _D), _F32)] * (3 - len(heads))
            y = jnp.concatenate(parts + [zpad], axis=0)
            if scale is not None:
                y = y * scale
            return y.astype(_BF16)

        q = stack(wq_ref, _QSCALE)
        k = stack(wk_ref)
        v = stack(wv_ref)
        sc = jnp.where(valid, _dot_nt(q, k), fill)
        m = jnp.max(sc, axis=1, keepdims=True)
        p = jnp.exp2(sc - m)
        l = jnp.sum(p, axis=1, keepdims=True)
        o = _dot(p.astype(_BF16), v) * (1.0 / l)
        for i, hh in enumerate(heads):
            oh = jnp.concatenate([o[i * _L:(i + 1) * _L], zpad], axis=0).astype(_BF16)
            t = _dot(oh, wo_ref[hh])
            acc = t if acc is None else acc + t
    out_ref[pl.ds(r0, _SEG), _DM:2 * _DM] = acc[0:_SEG].astype(out_ref.dtype)
    return acc[_SEG:_L].astype(_BF16).astype(_F32)


def _a_head(hh, xa_ref, ckv_ref, wq_ref, wuk_ref, wuv_ref, q_s, k_s, v_s, ctx_ref):
    q_s[...] = (_dot(xa_ref[...], wq_ref[hh]) * _QSCALE).astype(_BF16)
    k_s[...] = _dot(ckv_ref[...], wuk_ref[hh]).astype(_BF16)
    v_s[...] = _dot(ckv_ref[...], wuv_ref[hh]).astype(_BF16)
    r = jax.lax.broadcasted_iota(jnp.int32, (_BQ, _BQ), 0)
    c = jax.lax.broadcasted_iota(jnp.int32, (_BQ, _BQ), 1)
    tri = c <= r
    for qi in range(_S // _BQ):
        q = q_s[qi * _BQ:(qi + 1) * _BQ, :]
        m = l = acc = None
        for kj in range(qi + 1):
            k = k_s[kj * _BQ:(kj + 1) * _BQ, :]
            v = v_s[kj * _BQ:(kj + 1) * _BQ, :]
            sc = _dot_nt(q, k)
            if kj == qi:
                sc = jnp.where(tri, sc, _NEG_REF)
            mc = jnp.max(sc, axis=1, keepdims=True)
            if m is None:
                m = mc
                p = jnp.exp2(sc - m)
                l = jnp.sum(p, axis=1, keepdims=True)
                acc = _dot(p.astype(_BF16), v)
            else:
                mn = jnp.maximum(m, mc)
                alpha = jnp.exp2(m - mn)
                p = jnp.exp2(sc - mn)
                l = alpha * l + jnp.sum(p, axis=1, keepdims=True)
                acc = alpha * acc + _dot(p.astype(_BF16), v)
                m = mn
        ctx_ref[hh, qi * _BQ:(qi + 1) * _BQ, :] = (acc * (1.0 / l)).astype(_BF16)


def _kernel(xa_hbm, ckv_hbm, awq_hbm, awuk_hbm, awuv_hbm, awo_hbm,
            xb_hbm, mem_hbm, bwq_hbm, bwk_hbm, bwv_hbm, bwo_hbm,
            out_ref,
            xa, ckv, xb, mem0, awo, bwo, stage,
            awq, awuk, awuv, bwq, bwk, bwv,
            q_s, k_s, v_s, ctx, sems):
    def cp(src, dst, i):
        return pltpu.make_async_copy(src, dst, sems.at[i])

    plain = [(xa_hbm, xa), (ckv_hbm, ckv), (xb_hbm, xb), (mem_hbm, mem0), (awo_hbm, awo), (bwo_hbm, bwo)]
    for i, (s_, d_) in enumerate(plain):
        cp(s_, d_, i).start()
    rel = [(awq_hbm, awq, _DM), (awuk_hbm, awuk, _DC), (awuv_hbm, awuv, _DC),
           (bwq_hbm, bwq, _DM), (bwk_hbm, bwk, _DM), (bwv_hbm, bwv, _DM)]

    def stage_cp(i):
        src, _, k = rel[i]
        return cp(src, stage.at[i % 2, pl.ds(0, k)], 6 + i)

    stage_cp(0).start()
    for i, (_, dst, k) in enumerate(rel):
        if i + 1 < len(rel):
            stage_cp(i + 1).start()
        stage_cp(i).wait()
        _relayout(stage.at[i % 2], dst, k)
    for i, (s_, d_) in enumerate(plain):
        cp(s_, d_, i).wait()

    valid, fill = _b_bias(3)

    def a_body(hh, _):
        _a_head(hh, xa, ckv, awq, awuk, awuv, q_s, k_s, v_s, ctx)
    jax.lax.fori_loop(0, _H, a_body, None)

    def b_body(s, mem):
        return _b_step(s, mem, xb, bwq, bwk, bwv, bwo, out_ref, valid, fill)
    jax.lax.fori_loop(0, _NSEG, b_body, mem0[...].astype(_F32))

    def o_body(rb, _):
        r0 = pl.multiple_of(rb * 256, 256)
        acc = None
        for hh in range(_H):
            t = _dot(ctx[hh, pl.ds(r0, 256), :], awo[hh])
            acc = t if acc is None else acc + t
        out_ref[pl.ds(r0, 256), 0:_DM] = acc.astype(out_ref.dtype)
    jax.lax.fori_loop(0, _S // 256, o_body, None)


@jax.jit
def _run(A_x, A_c_kv, A_w_q, A_w_uk, A_w_uv, A_w_o, B_x, B_mem0, B_Wq, B_Wk, B_Wv, B_Wo):
    any_spec = pl.BlockSpec(memory_space=pl.ANY)
    vm = lambda shape: pltpu.VMEM(shape, _BF16)
    out = pl.pallas_call(
        _kernel,
        in_specs=[any_spec] * 12,
        out_specs=pl.BlockSpec(memory_space=pltpu.VMEM),
        out_shape=jax.ShapeDtypeStruct((_S, 2 * _DM), _BF16),
        scratch_shapes=[
            vm((_S, _DM)), vm((_S, _DC)), vm((_S, _DM)), vm((_MEM, _DM)),
            vm((_H, _D, _DM)), vm((_H, _D, _DM)), vm((2, _DM, _H, _D)),
            vm((_H, _DM, _D)), vm((_H, _DC, _D)), vm((_H, _DC, _D)),
            vm((_H, _DM, _D)), vm((_H, _DM, _D)), vm((_H, _DM, _D)),
            vm((_S, _D)), vm((_S, _D)), vm((_S, _D)), vm((_H, _S, _D)),
            pltpu.SemaphoreType.DMA((12,)),
        ],
        compiler_params=pltpu.CompilerParams(vmem_limit_bytes=120 * 1024 * 1024),
    )(A_x[0], A_c_kv[0], A_w_q, A_w_uk, A_w_uv, A_w_o, B_x[0], B_mem0[0], B_Wq, B_Wk, B_Wv, B_Wo)
    return out[None]


def pallas_concat_heads__compressed_kv_cla__memory_aug_recurrent_mem_tr__prompt_kernel(
    A_x, A_c_kv, A_w_q, A_w_uk, A_w_uv, A_w_o,
    B_x, B_mem0, B_Wq, B_Wk, B_Wv, B_Wo, B_seg_len,
):
    del B_seg_len
    return _run(A_x, A_c_kv, A_w_q, A_w_uk, A_w_uv, A_w_o, B_x, B_mem0, B_Wq, B_Wk, B_Wv, B_Wo)
```

```python
import jax
import jax.numpy as jnp
import numpy as np
import jax.experimental.pallas as pl
import jax.experimental.pallas.tpu as pltpu

_H = 32
_D = 128
_S = 2048
_DM = 576
_DC = 512
_MEM = 8
_SEG = 32
_NSEG = _S // _SEG
_L = _SEG + _MEM
_BQ = 256
_BK = 512
_LOG2E = 1.4426950408889634
_QSCALE = float(_D ** -0.5) * _LOG2E
_NEG_REF = -1000000000.0 * _LOG2E
_NEG_OUT = -1e30

_NT = (((1,), (1,)), ((), ()))
_F32 = jnp.float32
_BF16 = jnp.bfloat16
_U32 = jnp.uint32


def _dot(a, b):
    return jnp.dot(a, b, preferred_element_type=_F32)


def _dot_nt(a, b):
    return jax.lax.dot_general(a, b, _NT, preferred_element_type=_F32)


def _pack(x):
    return pltpu.bitcast(x, _U32)


def _unpack(x):
    return pltpu.bitcast(x, _BF16)


def _relayout(src_ref, dst_ref, k):
    def body(c, _):
        r = pl.multiple_of(c * 64, 64)
        r2 = pl.multiple_of(c * 32, 32)
        for u in range(4):
            blk = jnp.swapaxes(src_ref[pl.ds(r + u * 16, 16)], 0, 1)
            dst_ref[:, pl.ds(r2 + u * 8, 8), :] = _pack(blk)
    jax.lax.fori_loop(0, k // 64, body, None)


def _transpose_x(src_ref, dst_ref):
    def body(c, _):
        r = pl.multiple_of(c * 256, 256)
        r2 = pl.multiple_of(c * 128, 128)
        dst_ref[pl.ds(r2, 128), :] = _pack(src_ref[:, pl.ds(r, 256)].T)
    jax.lax.fori_loop(0, _S // 256, body, None)


def _transpose_wo(src_ref, dst_ref):
    def body(hh, _):
        dst_ref[hh] = _pack(src_ref[hh].T)
    jax.lax.fori_loop(0, _H, body, None)


def _copy_pack(src_ref, dst_ref):
    def body(c, _):
        r = pl.multiple_of(c * 256, 256)
        r2 = pl.multiple_of(c * 128, 128)
        dst_ref[pl.ds(r2, 128), :] = _pack(src_ref[pl.ds(r, 256), :])
    jax.lax.fori_loop(0, _S // 256, body, None)


def _b_bias():
    r = jax.lax.broadcasted_iota(jnp.int32, (128, 128), 0)
    c = jax.lax.broadcasted_iota(jnp.int32, (128, 128), 1)
    i32 = lambda b: b.astype(jnp.int32)
    rh = i32(r >= _L) + i32(r >= 2 * _L) + i32(r >= 3 * _L)
    ch = i32(c >= _L) + i32(c >= 2 * _L) + i32(c >= 3 * _L)
    ri = r - rh * _L
    ci = c - ch * _L
    same = rh == ch
    ok = jnp.logical_or(jnp.logical_or(ri >= _SEG, ci >= _SEG), ci <= ri)
    valid = jnp.logical_and(same, ok)
    fill = jnp.where(same, _NEG_REF, _NEG_OUT).astype(_F32)
    return valid, fill


def _b_step(s, st, xb_ref, wq_ref, wk_ref, wv_ref, wo_ref, out_ref, valid, fill):
    r0 = pl.multiple_of(s * _SEG, _SEG)
    r2 = pl.multiple_of(s * (_SEG // 2), _SEG // 2)
    xs = _unpack(xb_ref[pl.ds(r2, _SEG // 2), :])
    mem = st['mem']
    memb = jnp.concatenate([mem, jnp.zeros_like(mem)], axis=0).astype(_BF16)
    h = jnp.concatenate([xs, memb], axis=0)
    acc = None
    zpad = jnp.zeros((8, _D), _F32)
    groups = [list(range(g0, min(g0 + 3, _H))) for g0 in range(0, _H, 3)]

    def proj(w_ref, heads, scale=None):
        n = len(heads)
        y = _dot(h, jnp.concatenate([_unpack(w_ref[hh]) for hh in heads], axis=1))
        parts = [y[0:_L, i * _D:(i + 1) * _D] for i in range(n)]
        parts += [jnp.zeros((_L, _D), _F32)] * (3 - n)
        z = jnp.concatenate(parts + [zpad], axis=0)
        if scale is not None:
            z = z * scale
        return z.astype(_BF16)

    def outproj(o, heads):
        oh = jnp.concatenate(
            [jnp.concatenate([o[i * _L:(i + 1) * _L], zpad], axis=0) for i in range(len(heads))],
            axis=1).astype(_BF16)
        return _dot(oh, jnp.concatenate([_unpack(wo_ref[hh]) for hh in heads], axis=0))

    unit = 1.0 / (len(groups) * 4 * 2)
    q = proj(wq_ref, groups[0], _QSCALE)
    k = proj(wk_ref, groups[0])
    yield unit
    v = proj(wv_ref, groups[0])
    prev = None
    for gi, heads in enumerate(groups):
        nxt = groups[gi + 1] if gi + 1 < len(groups) else None
        sc = _dot_nt(q, k)
        qn = proj(wq_ref, nxt, _QSCALE) if nxt else None
        yield unit
        sc = jnp.where(valid, sc, fill)
        m = jnp.max(sc, axis=1, keepdims=True)
        p = jnp.exp2(sc - m)
        l = jnp.sum(p, axis=1, keepdims=True)
        kn = proj(wk_ref, nxt) if nxt else None
        yield unit
        if prev is not None:
            t = outproj(*prev)
            acc = t if acc is None else acc + t
        o = _dot(p.astype(_BF16), v)
        yield unit
        vn = proj(wv_ref, nxt) if nxt else None
        o = o * (1.0 / l)
        yield unit
        prev = (o, heads)
        q, k, v = qn, kn, vn
    acc = acc + outproj(*prev)
    out_ref[pl.ds(r0, _SEG), _DM:2 * _DM] = acc[0:_SEG].astype(out_ref.dtype)
    st['mem'] = acc[_SEG:_L].astype(_BF16).astype(_F32)


def _a_head(hh, first, xa_ref, ckv_ref, wq_ref, wuk_ref, wuv_ref, wo_ref, q_s, k_s, v_s, oacc):
    tot = 13 * _S + 144 * 256 + 5 * _S
    for (src, w_ref, dst, scale, kt) in ((ckv_ref, wuk_ref, k_s, None, 4), (ckv_ref, wuv_ref, v_s, None, 4),
                                         (xa_ref, wq_ref, q_s, _QSCALE, 5)):
        w = _unpack(w_ref[hh])
        for c in range(2):
            y = _dot(_unpack(src[c * 512:(c + 1) * 512, :]), w)
            if scale is not None:
                y = y * scale
            dst[c * 512:(c + 1) * 512, :] = _pack(y.astype(_BF16))
            yield kt * 1024 / tot
    r = jax.lax.broadcasted_iota(jnp.int32, (_BQ, _BQ), 0)
    c = jax.lax.broadcasted_iota(jnp.int32, (_BQ, _BQ), 1)
    tri = c <= r
    for qi in range(_S // _BQ):
        q = _unpack(q_s[qi * _BQ // 2:(qi + 1) * _BQ // 2, :])
        chunks = []
        k0 = 0
        while k0 < qi * _BQ:
            kk = min(_BK, qi * _BQ - k0)
            chunks.append((k0, kk, False))
            k0 += kk
        chunks.append((qi * _BQ, _BQ, True))
        m = l = acc = None
        for (k0, kk, diag) in chunks:
            k = _unpack(k_s[k0 // 2:(k0 + kk) // 2, :])
            v = _unpack(v_s[k0 // 2:(k0 + kk) // 2, :])
            sc = _dot_nt(q, k)
            yield _BQ * (kk // 128) / tot
            if diag:
                sc = jnp.where(tri, sc, _NEG_REF)
            mc = jnp.max(sc, axis=1, keepdims=True)
            if m is None:
                m = mc
                p = jnp.exp2(sc - m)
                l = jnp.sum(p, axis=1, keepdims=True)
                acc = _dot(p.astype(_BF16), v)
            else:
                mn = jnp.maximum(m, mc)
                alpha = jnp.exp2(m - mn)
                p = jnp.exp2(sc - mn)
                l = alpha * l + jnp.sum(p, axis=1, keepdims=True)
                acc = alpha * acc + _dot(p.astype(_BF16), v)
                m = mn
            yield _BQ * (kk // 128) / tot
        ctx = (acc * (1.0 / l)).astype(_BF16)
        t = _dot(ctx, _unpack(wo_ref[hh]))
        rows = slice(qi * _BQ, (qi + 1) * _BQ)
        if first:
            oacc[rows, :] = t
        else:
            oacc[rows, :] += t
        yield 5 * _BQ / tot


def _chain(*gens):
    for g in gens:
        yield from g


def _interleave(ga, gb):
    ca = cb = 0.0
    da = db = False
    end = object()
    while not (da and db):
        if db or (not da and ca <= cb):
            r = next(ga, end)
            if r is end:
                da = True
            else:
                ca += r
        else:
            r = next(gb, end)
            if r is end:
                db = True
            else:
                cb += r


def _kernel(xa_hbm, ckv_hbm, awq_hbm, awuk_hbm, awuv_hbm, awo_hbm,
            xb_hbm, mem_hbm, bwq_hbm, bwk_hbm, bwv_hbm, bwo_hbm,
            out_ref,
            xta, xtb, ckv0, mem0, wot, stage,
            xa, ckv, xb, awo, bwo,
            awq, awuk, awuv, bwq, bwk, bwv,
            q_s, k_s, v_s, oacc, sems):
    def cp(src, dst, i):
        return pltpu.make_async_copy(src, dst, sems.at[i])

    rel = [(awuk_hbm, awuk, _DC), (awuv_hbm, awuv, _DC), (awq_hbm, awq, _DM),
           (bwq_hbm, bwq, _DM), (bwk_hbm, bwk, _DM), (bwv_hbm, bwv, _DM)]

    def stage_cp(i):
        src, _, k = rel[i]
        return cp(src, stage.at[i % 3, pl.ds(0, k)], 6 + i)

    c_ckv = cp(ckv_hbm, ckv0, 0)
    c_xa = cp(xa_hbm, xta, 1)
    c_awo = cp(awo_hbm, wot.at[0], 2)
    c_bwo = cp(bwo_hbm, wot.at[1], 3)
    c_xb = cp(xb_hbm, xtb, 4)
    c_mem = cp(mem_hbm, mem0, 5)

    def do_rel(i):
        stage_cp(i).wait()
        _relayout(stage.at[i % 3], rel[i][1], rel[i][2])

    c_ckv.start(); stage_cp(0).start(); stage_cp(1).start()
    c_xa.start(); stage_cp(2).start(); c_awo.start()
    c_ckv.wait(); _copy_pack(ckv0, ckv)
    do_rel(0); stage_cp(3).start()
    do_rel(1); stage_cp(4).start()
    c_xa.wait(); _transpose_x(xta, xa)
    do_rel(2); stage_cp(5).start()
    c_bwo.start(); c_xb.start(); c_mem.start()
    c_awo.wait(); _transpose_wo(wot.at[0], awo)

    a_args = (xa, ckv, awq, awuk, awuv, awo, q_s, k_s, v_s, oacc)
    for _ in _a_head(0, True, *a_args):
        pass

    do_rel(3); do_rel(4); do_rel(5)
    c_bwo.wait(); _transpose_wo(wot.at[1], bwo)
    c_xb.wait(); _transpose_x(xtb, xb)
    c_mem.wait()

    valid, fill = _b_bias()
    b_args = (xb, bwq, bwk, bwv, bwo, out_ref, valid, fill)

    def ab_body(hh, mem):
        st = {'mem': mem}
        _interleave(_a_head(hh, False, *a_args),
                    _chain(_b_step(2 * hh - 2, st, *b_args), _b_step(2 * hh - 1, st, *b_args)))
        return st['mem']
    mem = jax.lax.fori_loop(1, _H, ab_body, mem0[...].astype(_F32))

    def b_body(s, mem):
        st = {'mem': mem}
        for _ in _b_step(s, st, *b_args):
            pass
        return st['mem']
    jax.lax.fori_loop(_NSEG - 2, _NSEG, b_body, mem)

    def o_body(rb, _):
        r0 = pl.multiple_of(rb * 256, 256)
        out_ref[pl.ds(r0, 256), 0:_DM] = oacc[pl.ds(r0, 256), :].astype(out_ref.dtype)
    jax.lax.fori_loop(0, _S // 256, o_body, None)


@jax.jit
def _run(A_x, A_c_kv, A_w_q, A_w_uk, A_w_uv, A_w_o, B_x, B_mem0, B_Wq, B_Wk, B_Wv, B_Wo):
    any_spec = pl.BlockSpec(memory_space=pltpu.HBM)
    vm = lambda shape: pltpu.VMEM(shape, _BF16)
    vu = lambda shape: pltpu.VMEM(shape, _U32)
    out = pl.pallas_call(
        _kernel,
        in_specs=[any_spec] * 12,
        out_specs=pl.BlockSpec(memory_space=pltpu.VMEM),
        out_shape=jax.ShapeDtypeStruct((_S, 2 * _DM), _BF16),
        scratch_shapes=[
            vm((_DM, _S)), vm((_DM, _S)), vm((_S, _DC)), vm((_MEM, _DM)),
            vm((2, _H, _DM, _D)), vm((3, _DM, _H, _D)),
            vu((_S // 2, _DM)), vu((_S // 2, _DC)), vu((_S // 2, _DM)),
            vu((_H, _D // 2, _DM)), vu((_H, _D // 2, _DM)),
            vu((_H, _DM // 2, _D)), vu((_H, _DC // 2, _D)), vu((_H, _DC // 2, _D)),
            vu((_H, _DM // 2, _D)), vu((_H, _DM // 2, _D)), vu((_H, _DM // 2, _D)),
            vu((_S // 2, _D)), vu((_S // 2, _D)), vu((_S // 2, _D)),
            pltpu.VMEM((_S, _DM), _F32),
            pltpu.SemaphoreType.DMA((12,)),
        ],
        compiler_params=pltpu.CompilerParams(vmem_limit_bytes=120 * 1024 * 1024),
    )(A_x[0].T, A_c_kv[0], A_w_q, A_w_uk, A_w_uv, jnp.swapaxes(A_w_o, 1, 2),
      B_x[0].T, B_mem0[0], B_Wq, B_Wk, B_Wv, jnp.swapaxes(B_Wo, 1, 2))
    return out[None]


def pallas_concat_heads__compressed_kv_cla__memory_aug_recurrent_mem_tr__prompt_kernel(
    A_x, A_c_kv, A_w_q, A_w_uk, A_w_uv, A_w_o,
    B_x, B_mem0, B_Wq, B_Wk, B_Wv, B_Wo, B_seg_len,
):
    del B_seg_len
    return _run(A_x, A_c_kv, A_w_q, A_w_uk, A_w_uv, A_w_o, B_x, B_mem0, B_Wq, B_Wk, B_Wv, B_Wo)
```

```python
import jax
import jax.numpy as jnp
import numpy as np
import jax.experimental.pallas as pl
import jax.experimental.pallas.tpu as pltpu

_H = 32
_D = 128
_S = 2048
_DM = 576
_DC = 512
_MEM = 8
_SEG = 32
_NSEG = _S // _SEG
_L = _SEG + _MEM
_BQ = 256
_BK = 1024
_LOG2E = 1.4426950408889634
_QSCALE = float(_D ** -0.5) * _LOG2E
_NEG_REF = -1000000000.0 * _LOG2E
_NEG_OUT = -1e30

_NT = (((1,), (1,)), ((), ()))
_F32 = jnp.float32
_BF16 = jnp.bfloat16
_U32 = jnp.uint32


def _dot(a, b):
    return jnp.dot(a, b, preferred_element_type=_F32)


def _dot_nt(a, b):
    return jax.lax.dot_general(a, b, _NT, preferred_element_type=_F32)


def _pack(x):
    return pltpu.bitcast(x, _U32)


def _unpack(x):
    return pltpu.bitcast(x, _BF16)


def _relayout(src_ref, dst_ref, k):
    def body(c, _):
        r = pl.multiple_of(c * 64, 64)
        r2 = pl.multiple_of(c * 32, 32)
        for u in range(4):
            blk = jnp.swapaxes(src_ref[pl.ds(r + u * 16, 16)], 0, 1)
            dst_ref[:, pl.ds(r2 + u * 8, 8), :] = _pack(blk)
    jax.lax.fori_loop(0, k // 64, body, None)


def _transpose_x(src_ref, dst_ref):
    def body(c, _):
        r = pl.multiple_of(c * 256, 256)
        r2 = pl.multiple_of(c * 128, 128)
        dst_ref[pl.ds(r2, 128), :] = _pack(src_ref[:, pl.ds(r, 256)].T)
    jax.lax.fori_loop(0, _S // 256, body, None)


def _transpose_wo(src_ref, dst_ref):
    def body(hh, _):
        dst_ref[hh] = _pack(src_ref[hh].T)
    jax.lax.fori_loop(0, _H, body, None)


def _copy_pack(src_ref, dst_ref):
    def body(c, _):
        r = pl.multiple_of(c * 256, 256)
        r2 = pl.multiple_of(c * 128, 128)
        dst_ref[pl.ds(r2, 128), :] = _pack(src_ref[pl.ds(r, 256), :])
    jax.lax.fori_loop(0, _S // 256, body, None)


def _b_bias():
    r = jax.lax.broadcasted_iota(jnp.int32, (128, 128), 0)
    c = jax.lax.broadcasted_iota(jnp.int32, (128, 128), 1)
    i32 = lambda b: b.astype(jnp.int32)
    rh = i32(r >= _L) + i32(r >= 2 * _L) + i32(r >= 3 * _L)
    ch = i32(c >= _L) + i32(c >= 2 * _L) + i32(c >= 3 * _L)
    ri = r - rh * _L
    ci = c - ch * _L
    same = rh == ch
    ok = jnp.logical_or(jnp.logical_or(ri >= _SEG, ci >= _SEG), ci <= ri)
    valid = jnp.logical_and(same, ok)
    fill = jnp.where(same, _NEG_REF, _NEG_OUT).astype(_F32)
    return valid, fill


def _b_step(s, st, xb_ref, wq_ref, wk_ref, wv_ref, wo_ref, out_ref, valid, fill):
    r0 = pl.multiple_of(s * _SEG, _SEG)
    r2 = pl.multiple_of(s * (_SEG // 2), _SEG // 2)
    xs = _unpack(xb_ref[pl.ds(r2, _SEG // 2), :])
    mem = st['mem']
    memb = jnp.concatenate([mem, jnp.zeros_like(mem)], axis=0).astype(_BF16)
    h = jnp.concatenate([xs, memb], axis=0)
    acc = None
    zpad = jnp.zeros((8, _D), _F32)
    groups = [list(range(g0, min(g0 + 3, _H))) for g0 in range(0, _H, 3)]

    def proj(w_ref, heads, scale=None):
        n = len(heads)
        y = _dot(h, jnp.concatenate([_unpack(w_ref[hh]) for hh in heads], axis=1))
        parts = [y[0:_L, i * _D:(i + 1) * _D] for i in range(n)]
        parts += [jnp.zeros((_L, _D), _F32)] * (3 - n)
        z = jnp.concatenate(parts + [zpad], axis=0)
        if scale is not None:
            z = z * scale
        return z.astype(_BF16)

    def outproj(o, heads):
        oh = jnp.concatenate(
            [jnp.concatenate([o[i * _L:(i + 1) * _L], zpad], axis=0) for i in range(len(heads))],
            axis=1).astype(_BF16)
        return _dot(oh, jnp.concatenate([_unpack(wo_ref[hh]) for hh in heads], axis=0))

    unit = 1.0 / (len(groups) * 4 * 2)
    q = proj(wq_ref, groups[0], _QSCALE)
    k = proj(wk_ref, groups[0])
    yield unit
    v = proj(wv_ref, groups[0])
    prev = None
    for gi, heads in enumerate(groups):
        nxt = groups[gi + 1] if gi + 1 < len(groups) else None
        sc = _dot_nt(q, k)
        qn = proj(wq_ref, nxt, _QSCALE) if nxt else None
        yield unit
        sc = jnp.where(valid, sc, fill)
        m = jnp.max(sc, axis=1, keepdims=True)
        p = jnp.exp2(sc - m)
        l = jnp.sum(p, axis=1, keepdims=True)
        kn = proj(wk_ref, nxt) if nxt else None
        yield unit
        if prev is not None:
            t = outproj(*prev)
            acc = t if acc is None else acc + t
        o = _dot(p.astype(_BF16), v)
        yield unit
        vn = proj(wv_ref, nxt) if nxt else None
        o = o * pl.reciprocal(l, approx=False)
        yield unit
        prev = (o, heads)
        q, k, v = qn, kn, vn
    acc = acc + outproj(*prev)
    out_ref[pl.ds(r0, _SEG), _DM:2 * _DM] = acc[0:_SEG].astype(out_ref.dtype)
    st['mem'] = acc[_SEG:_L].astype(_BF16).astype(_F32)


def _a_head(hh, first, xa_ref, ckv_ref, wq_ref, wuk_ref, wuv_ref, wo_ref, q_s, k_s, v_s, oacc):
    tot = 13 * _S + 144 * 256 + 5 * _S
    for (src, w_ref, dst, scale, kt) in ((ckv_ref, wuk_ref, k_s, None, 4), (ckv_ref, wuv_ref, v_s, None, 4),
                                         (xa_ref, wq_ref, q_s, _QSCALE, 5)):
        w = _unpack(w_ref[hh])
        for c in range(2):
            y = _dot(_unpack(src[c * 512:(c + 1) * 512, :]), w)
            if scale is not None:
                y = y * scale
            dst[c * 512:(c + 1) * 512, :] = _pack(y.astype(_BF16))
            yield kt * 1024 / tot
    wo = None
    r = jax.lax.broadcasted_iota(jnp.int32, (_BQ, _BQ), 0)
    c = jax.lax.broadcasted_iota(jnp.int32, (_BQ, _BQ), 1)
    tri = c <= r
    for qi in range(_S // _BQ):
        q = _unpack(q_s[qi * _BQ // 2:(qi + 1) * _BQ // 2, :])
        chunks = []
        k0 = 0
        while k0 < qi * _BQ:
            kk = min(_BK, qi * _BQ - k0)
            chunks.append((k0, kk, False))
            k0 += kk
        chunks.append((qi * _BQ, _BQ, True))
        m = l = acc = None
        for (k0, kk, diag) in chunks:
            k = _unpack(k_s[k0 // 2:(k0 + kk) // 2, :])
            v = _unpack(v_s[k0 // 2:(k0 + kk) // 2, :])
            sc = _dot_nt(q, k)
            yield _BQ * (kk // 128) / tot
            if diag:
                sc = jnp.where(tri, sc, _NEG_REF)
            mc = jnp.max(sc, axis=1, keepdims=True)
            if m is None:
                m = mc
                p = jnp.exp2(sc - m)
                l = jnp.sum(p, axis=1, keepdims=True)
                acc = _dot(p.astype(_BF16), v)
            else:
                mn = jnp.maximum(m, mc)
                alpha = jnp.exp2(m - mn)
                p = jnp.exp2(sc - mn)
                l = alpha * l + jnp.sum(p, axis=1, keepdims=True)
                acc = alpha * acc + _dot(p.astype(_BF16), v)
                m = mn
            yield _BQ * (kk // 128) / tot
        ctx = (acc * pl.reciprocal(l, approx=False)).astype(_BF16)
        if wo is None:
            wo = wo_ref[hh].T
        t = _dot(ctx, wo)
        rows = slice(qi * _BQ, (qi + 1) * _BQ)
        if first:
            oacc[rows, :] = t
        else:
            oacc[rows, :] += t
        yield 5 * _BQ / tot


def _chain(*gens):
    for g in gens:
        yield from g


def _interleave(ga, gb):
    ca = cb = 0.0
    da = db = False
    end = object()
    while not (da and db):
        if db or (not da and ca <= cb):
            r = next(ga, end)
            if r is end:
                da = True
            else:
                ca += r
        else:
            r = next(gb, end)
            if r is end:
                db = True
            else:
                cb += r


def _kernel(xa_hbm, ckv_hbm, awq_hbm, awuk_hbm, awuv_hbm, awo_hbm,
            xb_hbm, mem_hbm, bwq_hbm, bwk_hbm, bwv_hbm, bwo_hbm,
            out_ref,
            xta, xtb, ckv0, mem0, wot, stage,
            xa, ckv, xb, bwo,
            awq, awuk, awuv, bwq, bwk, bwv,
            q_s, k_s, v_s, oacc, sems):
    def cp(src, dst, i):
        return pltpu.make_async_copy(src, dst, sems.at[i])

    rel = [(awuk_hbm, awuk, _DC), (awuv_hbm, awuv, _DC), (awq_hbm, awq, _DM),
           (bwq_hbm, bwq, _DM), (bwk_hbm, bwk, _DM), (bwv_hbm, bwv, _DM)]

    def stage_cp(i):
        src, _, k = rel[i]
        return cp(src, stage.at[i, pl.ds(0, k)], 6 + i)

    c_ckv = cp(ckv_hbm, ckv0, 0)
    c_xa = cp(xa_hbm, xta, 1)
    c_awo = cp(awo_hbm, wot.at[0], 2)
    c_bwo = cp(bwo_hbm, wot.at[1], 3)
    c_xb = cp(xb_hbm, xtb, 4)
    c_mem = cp(mem_hbm, mem0, 5)

    def do_rel(i):
        stage_cp(i).wait()
        _relayout(stage.at[i], rel[i][1], rel[i][2])

    c_ckv.start(); stage_cp(0).start()

    a_args = (xa, ckv, awq, awuk, awuv, wot.at[0], q_s, k_s, v_s, oacc)
    g0 = _a_head(0, True, *a_args)
    c_ckv.wait(); _copy_pack(ckv0, ckv)
    stage_cp(0).wait()
    stage_cp(1).start(); c_xa.start()
    _relayout(stage.at[0], rel[0][1], rel[0][2])
    next(g0); next(g0)
    stage_cp(1).wait()
    stage_cp(2).start()
    _relayout(stage.at[1], rel[1][1], rel[1][2])
    next(g0); next(g0)
    c_xa.wait(); _transpose_x(xta, xa)
    stage_cp(2).wait()
    c_awo.start()
    _relayout(stage.at[2], rel[2][1], rel[2][2])
    next(g0); next(g0)
    c_awo.wait()
    stage_cp(3).start(); stage_cp(4).start()
    for _ in g0:
        pass
    stage_cp(5).start(); c_bwo.start(); c_xb.start(); c_mem.start()
    for _ in _a_head(1, False, *a_args):
        pass
    do_rel(3); do_rel(4); do_rel(5)
    c_bwo.wait(); _transpose_wo(wot.at[1], bwo)
    c_xb.wait(); _transpose_x(xtb, xb)
    c_mem.wait()

    valid, fill = _b_bias()
    b_args = (xb, bwq, bwk, bwv, bwo, out_ref, valid, fill)

    def ab_body(hh, mem):
        st = {'mem': mem}
        _interleave(_a_head(hh, False, *a_args),
                    _chain(_b_step(2 * hh - 4, st, *b_args), _b_step(2 * hh - 3, st, *b_args)))
        return st['mem']
    mem = jax.lax.fori_loop(2, _H, ab_body, mem0[...].astype(_F32))

    def b_body(s, mem):
        st = {'mem': mem}
        for _ in _b_step(s, st, *b_args):
            pass
        return st['mem']
    jax.lax.fori_loop(_NSEG - 4, _NSEG, b_body, mem)

    def o_body(rb, _):
        r0 = pl.multiple_of(rb * 256, 256)
        out_ref[pl.ds(r0, 256), 0:_DM] = oacc[pl.ds(r0, 256), :].astype(out_ref.dtype)
    jax.lax.fori_loop(0, _S // 256, o_body, None)


@jax.jit
def _run(A_x, A_c_kv, A_w_q, A_w_uk, A_w_uv, A_w_o, B_x, B_mem0, B_Wq, B_Wk, B_Wv, B_Wo):
    any_spec = pl.BlockSpec(memory_space=pltpu.HBM)
    vm = lambda shape: pltpu.VMEM(shape, _BF16)
    vu = lambda shape: pltpu.VMEM(shape, _U32)
    out = pl.pallas_call(
        _kernel,
        in_specs=[any_spec] * 12,
        out_specs=pl.BlockSpec(memory_space=pltpu.VMEM),
        out_shape=jax.ShapeDtypeStruct((_S, 2 * _DM), _BF16),
        scratch_shapes=[
            vm((_DM, _S)), vm((_DM, _S)), vm((_S, _DC)), vm((_MEM, _DM)),
            vm((2, _H, _DM, _D)), vm((6, _DM, _H, _D)),
            vu((_S // 2, _DM)), vu((_S // 2, _DC)), vu((_S // 2, _DM)),
            vu((_H, _D // 2, _DM)),
            vu((_H, _DM // 2, _D)), vu((_H, _DC // 2, _D)), vu((_H, _DC // 2, _D)),
            vu((_H, _DM // 2, _D)), vu((_H, _DM // 2, _D)), vu((_H, _DM // 2, _D)),
            vu((_S // 2, _D)), vu((_S // 2, _D)), vu((_S // 2, _D)),
            pltpu.VMEM((_S, _DM), _F32),
            pltpu.SemaphoreType.DMA((12,)),
        ],
        compiler_params=pltpu.CompilerParams(vmem_limit_bytes=120 * 1024 * 1024),
    )(A_x[0].T, A_c_kv[0], A_w_q, A_w_uk, A_w_uv, jnp.swapaxes(A_w_o, 1, 2),
      B_x[0].T, B_mem0[0], B_Wq, B_Wk, B_Wv, jnp.swapaxes(B_Wo, 1, 2))
    return out[None]


def pallas_concat_heads__compressed_kv_cla__memory_aug_recurrent_mem_tr__prompt_kernel(
    A_x, A_c_kv, A_w_q, A_w_uk, A_w_uv, A_w_o,
    B_x, B_mem0, B_Wq, B_Wk, B_Wv, B_Wo, B_seg_len,
):
    del B_seg_len
    return _run(A_x, A_c_kv, A_w_q, A_w_uk, A_w_uv, A_w_o, B_x, B_mem0, B_Wq, B_Wk, B_Wv, B_Wo)
```

```python
import jax
import jax.numpy as jnp
import numpy as np
import jax.experimental.pallas as pl
import jax.experimental.pallas.tpu as pltpu

_H = 32
_D = 128
_S = 2048
_DM = 576
_DC = 512
_MEM = 8
_SEG = 32
_NSEG = _S // _SEG
_L = _SEG + _MEM
_BQ = 256
_BK = 1024
_LOG2E = 1.4426950408889634
_QSCALE = float(_D ** -0.5) * _LOG2E
_NEG_REF = -1000000000.0 * _LOG2E
_NEG_OUT = -1e30

_NT = (((1,), (1,)), ((), ()))
_F32 = jnp.float32
_BF16 = jnp.bfloat16
_U32 = jnp.uint32


def _dot(a, b):
    return jnp.dot(a, b, preferred_element_type=_F32)


def _dot_nt(a, b):
    return jax.lax.dot_general(a, b, _NT, preferred_element_type=_F32)


def _pack(x):
    return pltpu.bitcast(x, _U32)


def _unpack(x):
    return pltpu.bitcast(x, _BF16)


def _relayout(src_ref, dst_ref, k):
    def body(c, _):
        r = pl.multiple_of(c * 64, 64)
        r2 = pl.multiple_of(c * 32, 32)
        for u in range(4):
            blk = jnp.swapaxes(src_ref[pl.ds(r + u * 16, 16)], 0, 1)
            dst_ref[:, pl.ds(r2 + u * 8, 8), :] = _pack(blk)
    jax.lax.fori_loop(0, k // 64, body, None)


def _transpose_x(src_ref, dst_ref):
    def body(c, _):
        r = pl.multiple_of(c * 256, 256)
        r2 = pl.multiple_of(c * 128, 128)
        dst_ref[pl.ds(r2, 128), :] = _pack(src_ref[:, pl.ds(r, 256)].T)
    jax.lax.fori_loop(0, _S // 256, body, None)


def _transpose_wo(src_ref, dst_ref):
    def body(hh, _):
        dst_ref[hh] = _pack(src_ref[hh].T)
    jax.lax.fori_loop(0, _H, body, None)


def _copy_pack(src_ref, dst_ref):
    def body(c, _):
        r = pl.multiple_of(c * 256, 256)
        r2 = pl.multiple_of(c * 128, 128)
        dst_ref[pl.ds(r2, 128), :] = _pack(src_ref[pl.ds(r, 256), :])
    jax.lax.fori_loop(0, _S // 256, body, None)


def _b_bias():
    r = jax.lax.broadcasted_iota(jnp.int32, (128, 128), 0)
    c = jax.lax.broadcasted_iota(jnp.int32, (128, 128), 1)
    i32 = lambda b: b.astype(jnp.int32)
    rh = i32(r >= _L) + i32(r >= 2 * _L) + i32(r >= 3 * _L)
    ch = i32(c >= _L) + i32(c >= 2 * _L) + i32(c >= 3 * _L)
    ri = r - rh * _L
    ci = c - ch * _L
    same = rh == ch
    ok = jnp.logical_or(jnp.logical_or(ri >= _SEG, ci >= _SEG), ci <= ri)
    valid = jnp.logical_and(same, ok)
    fill = jnp.where(same, _NEG_REF, _NEG_OUT).astype(_F32)
    return valid, fill


def _b_step(s, st, xb_ref, wq_ref, wk_ref, wv_ref, wo_ref, out_ref, valid, fill):
    r0 = pl.multiple_of(s * _SEG, _SEG)
    r2 = pl.multiple_of(s * (_SEG // 2), _SEG // 2)
    xs = _unpack(xb_ref[pl.ds(r2, _SEG // 2), :])
    mem = st['mem']
    memb = jnp.concatenate([mem, jnp.zeros_like(mem)], axis=0).astype(_BF16)
    h = jnp.concatenate([xs, memb], axis=0)
    acc = None
    zpad = jnp.zeros((8, _D), _F32)
    groups = [list(range(g0, min(g0 + 3, _H))) for g0 in range(0, _H, 3)]

    def proj(w_ref, heads, scale=None):
        n = len(heads)
        y = _dot(h, jnp.concatenate([_unpack(w_ref[hh]) for hh in heads], axis=1))
        parts = [y[0:_L, i * _D:(i + 1) * _D] for i in range(n)]
        parts += [jnp.zeros((_L, _D), _F32)] * (3 - n)
        z = jnp.concatenate(parts + [zpad], axis=0)
        if scale is not None:
            z = z * scale
        return z.astype(_BF16)

    def outproj(o, heads):
        oh = jnp.concatenate(
            [jnp.concatenate([o[i * _L:(i + 1) * _L], zpad], axis=0) for i in range(len(heads))],
            axis=1).astype(_BF16)
        return _dot(oh, jnp.concatenate([_unpack(wo_ref[hh]) for hh in heads], axis=0))

    unit = 1.0 / (len(groups) * 4 * 2)
    q = proj(wq_ref, groups[0], _QSCALE)
    k = proj(wk_ref, groups[0])
    yield unit
    v = proj(wv_ref, groups[0])
    prev = None
    for gi, heads in enumerate(groups):
        nxt = groups[gi + 1] if gi + 1 < len(groups) else None
        sc = _dot_nt(q, k)
        qn = proj(wq_ref, nxt, _QSCALE) if nxt else None
        yield unit
        sc = jnp.where(valid, sc, fill)
        m = jnp.max(sc, axis=1, keepdims=True)
        p = jnp.exp2(sc - m)
        l = jnp.sum(p, axis=1, keepdims=True)
        kn = proj(wk_ref, nxt) if nxt else None
        yield unit
        if prev is not None:
            t = outproj(*prev)
            acc = t if acc is None else acc + t
        o = _dot(p.astype(_BF16), v)
        yield unit
        vn = proj(wv_ref, nxt) if nxt else None
        o = o * pl.reciprocal(l, approx=False)
        yield unit
        prev = (o, heads)
        q, k, v = qn, kn, vn
    acc = acc + outproj(*prev)
    out_ref[pl.ds(r0, _SEG), _DM:2 * _DM] = acc[0:_SEG].astype(out_ref.dtype)
    st['mem'] = acc[_SEG:_L].astype(_BF16).astype(_F32)


def _a_head(hh, first, xa_ref, ckv_ref, wq_ref, wuk_ref, wuv_ref, wo_ref, q_s, k_s, v_s, oacc):
    tot = 13 * _S + 144 * 256 + 5 * _S
    for (src, w_ref, dst, scale, kt) in ((ckv_ref, wuk_ref, k_s, None, 4), (ckv_ref, wuv_ref, v_s, None, 4),
                                         (xa_ref, wq_ref, q_s, _QSCALE, 5)):
        w = _unpack(w_ref[hh])
        for c in range(2):
            y = _dot(_unpack(src[c * 512:(c + 1) * 512, :]), w)
            if scale is not None:
                y = y * scale
            dst[c * 512:(c + 1) * 512, :] = _pack(y.astype(_BF16))
            yield kt * 1024 / tot
    wo = None
    r = jax.lax.broadcasted_iota(jnp.int32, (_BQ, _BQ), 0)
    c = jax.lax.broadcasted_iota(jnp.int32, (_BQ, _BQ), 1)
    tri = c <= r
    for qi in range(_S // _BQ):
        q = _unpack(q_s[qi * _BQ // 2:(qi + 1) * _BQ // 2, :])
        chunks = []
        k0 = 0
        while k0 < qi * _BQ:
            kk = min(_BK, qi * _BQ - k0)
            chunks.append((k0, kk, False))
            k0 += kk
        chunks.append((qi * _BQ, _BQ, True))
        m = l = acc = None
        for (k0, kk, diag) in chunks:
            k = _unpack(k_s[k0 // 2:(k0 + kk) // 2, :])
            v = _unpack(v_s[k0 // 2:(k0 + kk) // 2, :])
            if diag:
                hb = _BQ // 2
                sc = jnp.concatenate([
                    jnp.concatenate([_dot_nt(q[:hb], k[:hb]), jnp.full((hb, hb), _NEG_REF, _F32)], axis=1),
                    _dot_nt(q[hb:], k)], axis=0)
                pv = lambda pb, v: jnp.concatenate([_dot(pb[:hb, :hb], v[:hb]), _dot(pb[hb:], v)], axis=0)
            else:
                sc = _dot_nt(q, k)
                pv = _dot
            yield _BQ * (kk // 128) / tot
            if diag:
                sc = jnp.where(tri, sc, _NEG_REF)
            mc = jnp.max(sc, axis=1, keepdims=True)
            if m is None:
                m = mc
                p = jnp.exp2(sc - m)
                l = jnp.sum(p, axis=1, keepdims=True)
                acc = pv(p.astype(_BF16), v)
            else:
                mn = jnp.maximum(m, mc)
                alpha = jnp.exp2(m - mn)
                p = jnp.exp2(sc - mn)
                l = alpha * l + jnp.sum(p, axis=1, keepdims=True)
                acc = alpha * acc + pv(p.astype(_BF16), v)
                m = mn
            yield _BQ * (kk // 128) / tot
        ctx = (acc * pl.reciprocal(l, approx=False)).astype(_BF16)
        if wo is None:
            wo = wo_ref[hh].T
        t = _dot(ctx, wo)
        rows = slice(qi * _BQ, (qi + 1) * _BQ)
        if first:
            oacc[rows, :] = t
        else:
            oacc[rows, :] += t
        yield 5 * _BQ / tot


def _chain(*gens):
    for g in gens:
        yield from g


def _interleave(ga, gb):
    ca = cb = 0.0
    da = db = False
    end = object()
    while not (da and db):
        if db or (not da and ca <= cb):
            r = next(ga, end)
            if r is end:
                da = True
            else:
                ca += r
        else:
            r = next(gb, end)
            if r is end:
                db = True
            else:
                cb += r


def _kernel(xa_hbm, ckv_hbm, awq_hbm, awuk_hbm, awuv_hbm, awo_hbm,
            xb_hbm, mem_hbm, bwq_hbm, bwk_hbm, bwv_hbm, bwo_hbm,
            out_ref,
            xta, xtb, ckv0, mem0, wot, stage,
            xa, ckv, xb, bwo,
            awq, awuk, awuv, bwq, bwk, bwv,
            q_s, k_s, v_s, oacc, sems):
    def cp(src, dst, i):
        return pltpu.make_async_copy(src, dst, sems.at[i])

    rel = [(awuk_hbm, awuk, _DC), (awuv_hbm, awuv, _DC), (awq_hbm, awq, _DM),
           (bwq_hbm, bwq, _DM), (bwk_hbm, bwk, _DM), (bwv_hbm, bwv, _DM)]

    def stage_cp(i):
        src, _, k = rel[i]
        return cp(src, stage.at[i, pl.ds(0, k)], 6 + i)

    c_ckv = cp(ckv_hbm, ckv0, 0)
    c_xa = cp(xa_hbm, xta, 1)
    c_awo = cp(awo_hbm, wot.at[0], 2)
    c_bwo = cp(bwo_hbm, wot.at[1], 3)
    c_xb = cp(xb_hbm, xtb, 4)
    c_mem = cp(mem_hbm, mem0, 5)

    def do_rel(i):
        stage_cp(i).wait()
        _relayout(stage.at[i], rel[i][1], rel[i][2])

    c_ckv.start(); stage_cp(0).start()

    a_args = (xa, ckv, awq, awuk, awuv, wot.at[0], q_s, k_s, v_s, oacc)
    g0 = _a_head(0, True, *a_args)
    c_ckv.wait(); _copy_pack(ckv0, ckv)
    stage_cp(0).wait()
    stage_cp(1).start(); c_xa.start()
    _relayout(stage.at[0], rel[0][1], rel[0][2])
    next(g0); next(g0)
    stage_cp(1).wait()
    stage_cp(2).start()
    _relayout(stage.at[1], rel[1][1], rel[1][2])
    next(g0); next(g0)
    c_xa.wait(); _transpose_x(xta, xa)
    stage_cp(2).wait()
    c_awo.start()
    _relayout(stage.at[2], rel[2][1], rel[2][2])
    next(g0); next(g0)
    c_awo.wait()
    stage_cp(3).start(); stage_cp(4).start()
    for _ in g0:
        pass
    stage_cp(5).start(); c_bwo.start(); c_xb.start(); c_mem.start()
    for _ in _a_head(1, False, *a_args):
        pass
    do_rel(3); do_rel(4); do_rel(5)
    c_bwo.wait(); _transpose_wo(wot.at[1], bwo)
    c_xb.wait(); _transpose_x(xtb, xb)
    c_mem.wait()

    valid, fill = _b_bias()
    b_args = (xb, bwq, bwk, bwv, bwo, out_ref, valid, fill)

    def ab_body(hh, mem):
        st = {'mem': mem}
        _interleave(_a_head(hh, False, *a_args),
                    _chain(_b_step(2 * hh - 4, st, *b_args), _b_step(2 * hh - 3, st, *b_args)))
        return st['mem']
    mem = jax.lax.fori_loop(2, _H, ab_body, mem0[...].astype(_F32))

    def b_body(s, mem):
        st = {'mem': mem}
        for _ in _b_step(s, st, *b_args):
            pass
        return st['mem']
    jax.lax.fori_loop(_NSEG - 4, _NSEG, b_body, mem)

    def o_body(rb, _):
        r0 = pl.multiple_of(rb * 256, 256)
        out_ref[pl.ds(r0, 256), 0:_DM] = oacc[pl.ds(r0, 256), :].astype(out_ref.dtype)
    jax.lax.fori_loop(0, _S // 256, o_body, None)


@jax.jit
def _run(A_x, A_c_kv, A_w_q, A_w_uk, A_w_uv, A_w_o, B_x, B_mem0, B_Wq, B_Wk, B_Wv, B_Wo):
    any_spec = pl.BlockSpec(memory_space=pltpu.HBM)
    vm = lambda shape: pltpu.VMEM(shape, _BF16)
    vu = lambda shape: pltpu.VMEM(shape, _U32)
    out = pl.pallas_call(
        _kernel,
        in_specs=[any_spec] * 12,
        out_specs=pl.BlockSpec(memory_space=pltpu.VMEM),
        out_shape=jax.ShapeDtypeStruct((_S, 2 * _DM), _BF16),
        scratch_shapes=[
            vm((_DM, _S)), vm((_DM, _S)), vm((_S, _DC)), vm((_MEM, _DM)),
            vm((2, _H, _DM, _D)), vm((6, _DM, _H, _D)),
            vu((_S // 2, _DM)), vu((_S // 2, _DC)), vu((_S // 2, _DM)),
            vu((_H, _D // 2, _DM)),
            vu((_H, _DM // 2, _D)), vu((_H, _DC // 2, _D)), vu((_H, _DC // 2, _D)),
            vu((_H, _DM // 2, _D)), vu((_H, _DM // 2, _D)), vu((_H, _DM // 2, _D)),
            vu((_S // 2, _D)), vu((_S // 2, _D)), vu((_S // 2, _D)),
            pltpu.VMEM((_S, _DM), _F32),
            pltpu.SemaphoreType.DMA((12,)),
        ],
        compiler_params=pltpu.CompilerParams(vmem_limit_bytes=120 * 1024 * 1024),
    )(A_x[0].T, A_c_kv[0], A_w_q, A_w_uk, A_w_uv, jnp.swapaxes(A_w_o, 1, 2),
      B_x[0].T, B_mem0[0], B_Wq, B_Wk, B_Wv, jnp.swapaxes(B_Wo, 1, 2))
    return out[None]


def pallas_concat_heads__compressed_kv_cla__memory_aug_recurrent_mem_tr__prompt_kernel(
    A_x, A_c_kv, A_w_q, A_w_uk, A_w_uv, A_w_o,
    B_x, B_mem0, B_Wq, B_Wk, B_Wv, B_Wo, B_seg_len,
):
    del B_seg_len
    return _run(A_x, A_c_kv, A_w_q, A_w_uk, A_w_uv, A_w_o, B_x, B_mem0, B_Wq, B_Wk, B_Wv, B_Wo)
```
